```python
import jax
import jax.numpy as jnp

def _softmax(x, axis=-1):
    return jax.nn.softmax(x, axis=axis)
def _gelu(x):
    return jax.nn.gelu(x, approximate=True)
def _silu(x):
    return jax.nn.silu(x)
def _sigmoid(x):
    return jax.nn.sigmoid(x)
def _layernorm(x, axis=-1, eps=1e-5):
    m = jnp.mean(x, axis=axis, keepdims=True)
    v = jnp.var(x, axis=axis, keepdims=True)
    return (x - m) / jnp.sqrt(v + eps)
def _scatter_add(tgt, idx, src, axis=0):
    return tgt.at[idx].add(src)
def _segment_sum(src, seg, n):
    return jax.ops.segment_sum(src, seg, n)
class _Rng:
    def __init__(self, key):
        self._k = key
    def _next(self):
        self._k, sub = jax.random.split(self._k)
        return sub
    def normal(self, shape):
        return jax.random.normal(self._next(), shape, dtype=jnp.bfloat16)
    def randint(self, lo, hi, shape):
        return jax.random.randint(self._next(), shape, lo, hi, dtype=jnp.int32)
    def uniform(self, shape, lo=0.0, hi=1.0):
        return jax.random.uniform(self._next(), shape, jnp.bfloat16, lo, hi)
    def permutation(self, n):
        return jax.random.permutation(self._next(), n)


kernel_name = 'recurrent_scan__compressed_kv_cla__moe_arch_mod__decode'

def setup_inputs():
    _rng = _Rng(jax.random.key(int.from_bytes(__import__("os").urandom(4), "little")))
    _w = (lambda a: (lambda t: t.astype(jnp.bfloat16) if jnp.issubdtype(t.dtype, jnp.floating) else t)(jnp.asarray(a)))
    def _A_setup():
        B, H, Sq, Sk, D, M = 4, 32, 1, 4096, 128, 576
        Dc = 4 * D
        return {
            "x": _w((lambda *s: _rng.normal(s) * 0.05)(B, Sq, M)),
            "c_kv": _w((lambda *s: _rng.normal(s) * 0.05)(B, Sk, Dc)),
            "w_q": _w((lambda *s: _rng.normal(s) * 0.05)(M, H, D) * (M ** -0.5)),
            "w_uk": _w((lambda *s: _rng.normal(s) * 0.05)(Dc, H, D) * (Dc ** -0.5)),
            "w_uv": _w((lambda *s: _rng.normal(s) * 0.05)(Dc, H, D) * (Dc ** -0.5)),
            "w_o": _w((lambda *s: _rng.normal(s) * 0.05)(H, D, M) * ((H * D) ** -0.5)),
        }
    _A_in = _A_setup()

    def _B_setup():
        B, S, D, F, C = 4, 1, 576, 4608, 1
        return {
            "x": _w((lambda *s: _rng.normal(s) * 0.05)(B, S, D)),
            "w_r": _w((lambda *s: _rng.normal(s) * 0.05)(D)),
            "w_gate": _w((lambda *s: _rng.normal(s) * 0.05)(D, F)),
            "w_up": _w((lambda *s: _rng.normal(s) * 0.05)(D, F)),
            "w_down": _w((lambda *s: _rng.normal(s) * 0.05)(F, D)),
        }
    _B_in = _B_setup()

    return {
        "A_x": _A_in["x"],
        "A_c_kv": _A_in["c_kv"],
        "A_w_q": _A_in["w_q"],
        "A_w_uk": _A_in["w_uk"],
        "A_w_uv": _A_in["w_uv"],
        "A_w_o": _A_in["w_o"],
        "B_x": _B_in["x"],
        "B_w_r": _B_in["w_r"],
        "B_w_gate": _B_in["w_gate"],
        "B_w_up": _B_in["w_up"],
        "B_w_down": _B_in["w_down"],
    }

def reference(A_x, A_c_kv, A_w_q, A_w_uk, A_w_uv, A_w_o, B_x, B_w_r, B_w_gate, B_w_up, B_w_down):
    def _A_ref(x, c_kv, w_q, w_uk, w_uv, w_o):
        B, Sq, M = x.shape[0], x.shape[1], x.shape[2]
        Sk = c_kv.shape[1]
        H, D = w_q.shape[1], w_q.shape[2]
        q = jnp.einsum("bqm,mhd->bhqd", x, w_q)
        k = jnp.einsum("bkc,chd->bhkd", c_kv, w_uk)
        v = jnp.einsum("bkc,chd->bhkd", c_kv, w_uv)
        scores = jnp.einsum("bhqd,bhkd->bhqk", q, k) * (D ** -0.5)
        off = Sk - Sq
        qi = jnp.arange(Sq)[:, None]
        kj = jnp.arange(Sk)[None, :]
        cmask = kj <= (qi + off)
        scores = jnp.where(cmask[None, None], scores, -1e9)
        p = _softmax(scores, axis=-1)
        ctx = jnp.einsum("bhqk,bhkd->bhqd", p, v)
        return jnp.einsum("bhqd,hdm->bqm", ctx, w_o)

    def _B_ref(x, w_r, w_gate, w_up, w_down):
        B, S, D = x.shape
        C = 1
        r = x @ w_r
        idx = jnp.argsort(-r, axis=-1)[:, :C]
        idx_e = jnp.repeat(idx.reshape(B, C, 1), D, axis=2)
        x_sel = jnp.take_along_axis(x, idx_e, axis=1)
        g = _silu(x_sel @ w_gate)
        u = x_sel @ w_up
        y = (g * u) @ w_down
        r_sel = _sigmoid(jnp.take_along_axis(r, idx, axis=1))
        y = y * r_sel.reshape(B, C, 1)
        b_off = (jnp.arange(B) * S).reshape(B, 1)
        flat_idx = (idx + b_off).reshape(B * C)
        zero = (x * 0.0).reshape(B * S, D)
        upd = _scatter_add(zero, flat_idx, y.reshape(B * C, D), axis=0)
        return x + upd.reshape(B, S, D)

    x = A_x
    xn = _layernorm(x, axis=-1)
    s = _A_ref(xn, A_c_kv, A_w_q, A_w_uk, A_w_uv, A_w_o)
    g = _silu(_B_ref(xn, B_w_r, B_w_gate, B_w_up, B_w_down))
    return x + s * g
```

```python
import jax
import jax.numpy as jnp
from jax import lax
import jax.experimental.pallas as pl
import jax.experimental.pallas.tpu as pltpu

bf16, f32, i32 = jnp.bfloat16, jnp.float32, jnp.int32
_NT = (((1,), (1,)), ((), ()))

B, H, D, M, SK, DC, F = 4, 32, 128, 576, 4096, 512, 4608
G = 16


def _dot(a, b):
    return jnp.dot(a, b, preferred_element_type=f32)


def _dot_nt(a, b):
    return lax.dot_general(a, b, _NT, preferred_element_type=f32)


def _sigmoid(v):
    return 1.0 / (1.0 + jnp.exp(-v))


def _make(do_dma=True, do_compute=True, wo_split=(2,) * 15 + (1, 1), nocheck=True, debug=False):
    n_wo = len(wo_split)

    def kernel(x_h, ckv_h, wq_h, wuk_h, wuv_h, wo_h, wr_h, wg_h, wu_h, wd_h,
               *rest):
        if debug:
            o_ref, dbg_s, dbg_g = rest[:3]
            rest = rest[3:]
        else:
            o_ref = rest[0]
            rest = rest[1:]
        (x_v, wr_v, ckv_v, wq_v, wuk_v, wuv_v, wo_v, wg_v, wu_v, wd_v,
         e_v, et_v, xq_v, qa_v, lat_v, ctx_v, lhs_v, sems) = rest

        cp_x = pltpu.make_async_copy(x_h, x_v, sems.at[0])
        cp_wr = pltpu.make_async_copy(wr_h, wr_v, sems.at[1])
        cp_wq = pltpu.make_async_copy(wq_h, wq_v, sems.at[2])
        cp_wuk = pltpu.make_async_copy(wuk_h, wuk_v, sems.at[3])

        def cp_ckv(b):
            return pltpu.make_async_copy(ckv_h.at[b], ckv_v.at[b], sems.at[4 + b])

        cp_wuv = pltpu.make_async_copy(wuv_h, wuv_v, sems.at[8])
        cp_wg = pltpu.make_async_copy(wg_h, wg_v, sems.at[9])
        cp_wu = pltpu.make_async_copy(wu_h, wu_v, sems.at[10])
        cp_wd = pltpu.make_async_copy(wd_h, wd_v, sems.at[11])
        cp_wo = []
        h0 = 0
        for i, n in enumerate(wo_split):
            cp_wo.append(pltpu.make_async_copy(
                wo_h.at[pl.ds(h0, n)], wo_v.at[pl.ds(h0, n)], sems.at[12 + i]))
            h0 += n
        if do_dma:
            for cp in [cp_x, cp_wr, cp_wq, cp_wuk] + [cp_ckv(b) for b in range(B)] + [
                    cp_wuv, cp_wg, cp_wu, cp_wd] + cp_wo:
                cp.start()

        def wait(cp):
            if do_dma:
                cp.wait()

        if not do_compute:
            for cp in [cp_x, cp_wr, cp_wq, cp_wuk] + [cp_ckv(b) for b in range(B)] + [
                    cp_wuv, cp_wg, cp_wu, cp_wd] + cp_wo:
                wait(cp)
            o_ref[...] = x_v[...]
            return

        row = lax.broadcasted_iota(i32, (128, 128 * G), 0)
        col = lax.broadcasted_iota(i32, (128, 128 * G), 1)
        e_v[...] = jnp.where(row == (col >> 4), 1.0, 0.0).astype(bf16)
        row = lax.broadcasted_iota(i32, (128 * G, 128), 0)
        col = lax.broadcasted_iota(i32, (128 * G, 128), 1)
        et_v[...] = jnp.where(col == (row >> 4), 1.0, 0.0).astype(bf16)

        def head_mask(shape):
            r = lax.broadcasted_iota(i32, shape, 0)
            c = lax.broadcasted_iota(i32, shape, 1)
            return (r & (G - 1)) == (c & (G - 1))

        wait(cp_x)
        wait(cp_wr)
        x = x_v[...].astype(f32)
        mu = jnp.mean(x, axis=-1, keepdims=True)
        xc = x - mu
        var = jnp.mean(xc * xc, axis=-1, keepdims=True)
        xn = (xc / jnp.sqrt(var + 1e-5)).astype(bf16).astype(f32)
        wr = wr_v[...].astype(f32).reshape(1, M)
        r = jnp.sum(xn * wr, axis=-1, keepdims=True)
        xn8 = jnp.concatenate([xn, jnp.zeros_like(xn)], axis=0).astype(bf16)

        for blk in range(5):
            n = min(128, M - blk * 128)
            xe = _dot(xn8[:, blk * 128: blk * 128 + n], e_v[0:n, 0:n * G])
            msk = head_mask((G, n * G))
            for b in range(B):
                v = jnp.where(msk, jnp.broadcast_to(xe[b:b + 1], (G, n * G)), 0.0)
                xq_v[b * G:(b + 1) * G, blk * 128 * G: (blk * 128 + n) * G] = v.astype(bf16)

        wait(cp_wq)
        KB = 64

        def q_body(i, acc):
            m0 = pl.multiple_of(i * KB, KB)
            xl = xq_v[:, pl.ds(pl.multiple_of(i * KB * G, KB * G), KB * G)]
            out = []
            for g in range(2):
                w = wq_v[pl.ds(m0, KB), g * G:(g + 1) * G, :].reshape(KB * G, D)
                out.append(acc[g] + _dot(xl, w))
            return tuple(out)

        z = jnp.zeros((B * G, D), f32)
        q0, q1 = lax.fori_loop(0, M // KB, q_body, (z, z))
        q = (q0.astype(bf16), q1.astype(bf16))

        wait(cp_wuk)

        def qa_body(i, _):
            c0 = pl.multiple_of(i * 128, 128)
            t = []
            for g in range(2):
                w = wuk_v[pl.ds(c0, 128), g * G:(g + 1) * G, :].reshape(128 * G, D)
                t.append(_dot_nt(q[g], w))
            t = jnp.concatenate(t, axis=0)
            t = jnp.where(head_mask(t.shape), t, 0.0).astype(bf16)
            qa_v[:, pl.ds(c0, 128)] = _dot(t, et_v[...]).astype(bf16)
            return 0

        lax.fori_loop(0, DC // 128, qa_body, 0)

        def attn_body(b, _):
            wait(cp_ckv(b))
            r0 = pl.multiple_of(b * G, G)
            r1 = pl.multiple_of(B * G + b * G, G)
            qa = jnp.concatenate([qa_v[pl.ds(r0, G), :], qa_v[pl.ds(r1, G), :]], axis=0)
            s = _dot_nt(qa, ckv_v[b]) * (D ** -0.5)
            mx = jnp.max(s, axis=-1, keepdims=True)
            p = jnp.exp(s - mx)
            l = jnp.sum(p, axis=-1, keepdims=True)
            lat = _dot(p.astype(bf16), ckv_v[b]) / l
            lat = lat.astype(bf16)
            lat_v[pl.ds(r0, G), :] = lat[:G]
            lat_v[pl.ds(r1, G), :] = lat[G:]
            return 0

        lax.fori_loop(0, B, attn_body, 0)

        wait(cp_wuv)

        def ctx_body(i, acc):
            c0 = pl.multiple_of(i * 128, 128)
            xe = _dot(lat_v[:, pl.ds(c0, 128)], e_v[...])
            xe = jnp.where(head_mask(xe.shape), xe, 0.0).astype(bf16)
            out = []
            for g in range(2):
                w = wuv_v[pl.ds(c0, 128), g * G:(g + 1) * G, :].reshape(128 * G, D)
                out.append(acc[g] + _dot(xe[g * B * G:(g + 1) * B * G], w))
            return tuple(out)

        c0_, c1_ = lax.fori_loop(0, DC // 128, ctx_body, (z, z))
        ctx_v[0:B * G, :] = c0_
        ctx_v[B * G:, :] = c1_
        top = lax.broadcasted_iota(i32, (8, D), 0) < B
        for j in range(G):
            v = ctx_v[pl.ds(j, 8, stride=G), :]
            lhs_v[j] = jnp.where(top, v, 0.0).astype(bf16)
            lhs_v[G + j] = jnp.where(top, pltpu.roll(v, B, 0), 0.0).astype(bf16)

        wait(cp_wg)
        gate = _dot(xn8, wg_v[...])
        wait(cp_wu)
        up = _dot(xn8, wu_v[...])
        hid = (gate * _sigmoid(gate) * up).astype(bf16)
        wait(cp_wd)
        y = _dot_nt(hid, wd_v[...])[:B] * _sigmoid(r)
        z2 = xn + (xn * 0.0 + y)
        gfin = z2 * _sigmoid(z2)

        acc = jnp.zeros((8, M), f32)
        h0 = 0
        for i, n in enumerate(wo_split):
            wait(cp_wo[i])
            if n > 2:
                def o_body(h, a):
                    return a + _dot_nt(lhs_v[h], wo_v[h])
                acc = lax.fori_loop(h0, h0 + n, o_body, acc)
            else:
                for h in range(h0, h0 + n):
                    acc = acc + _dot_nt(lhs_v[h], wo_v[h])
            h0 += n
        s_out = acc[:B]
        o_ref[...] = (x + s_out * gfin).astype(o_ref.dtype)
        if debug:
            dbg_s[...] = s_out
            dbg_g[...] = gfin

    def fn(A_x, A_c_kv, A_w_q, A_w_uk, A_w_uv, A_w_o, B_x, B_w_r, B_w_gate, B_w_up, B_w_down):
        del B_x
        hbm = pl.BlockSpec(memory_space=pltpu.HBM)
        out_shape = jax.ShapeDtypeStruct((B, M), A_x.dtype)
        if debug:
            out_shape = (out_shape, jax.ShapeDtypeStruct((B, M), f32), jax.ShapeDtypeStruct((B, M), f32))
        out = pl.pallas_call(
            kernel,
            in_specs=[hbm] * 10,
            out_shape=out_shape,
            scratch_shapes=[
                pltpu.VMEM((B, M), bf16),
                pltpu.VMEM((M,), bf16),
                pltpu.VMEM((B, SK, DC), bf16),
                pltpu.VMEM((M, H, D), bf16),
                pltpu.VMEM((DC, H, D), bf16),
                pltpu.VMEM((DC, H, D), bf16),
                pltpu.VMEM((H, M, D), bf16),
                pltpu.VMEM((M, F), bf16),
                pltpu.VMEM((M, F), bf16),
                pltpu.VMEM((M, F), bf16),
                pltpu.VMEM((128, 128 * G), bf16),
                pltpu.VMEM((128 * G, 128), bf16),
                pltpu.VMEM((B * G, M * G), bf16),
                pltpu.VMEM((B * H, DC), bf16),
                pltpu.VMEM((B * H, DC), bf16),
                pltpu.VMEM((B * H, D), f32),
                pltpu.VMEM((H, 8, D), bf16),
                pltpu.SemaphoreType.DMA((12 + n_wo,)),
            ],
            compiler_params=pltpu.CompilerParams(
                vmem_limit_bytes=100 * 1024 * 1024,
                disable_semaphore_checks=nocheck,
            ),
        )(
            A_x.reshape(B, M), A_c_kv, A_w_q, A_w_uk, A_w_uv,
            jnp.transpose(A_w_o, (0, 2, 1)), B_w_r, B_w_gate, B_w_up, B_w_down.T,
        )
        if debug:
            return out[0].reshape(B, 1, M), out[1], out[2]
        return out.reshape(B, 1, M)

    return fn


@jax.jit
def pallas_recurrent_scan__compressed_kv_cla__moe_arch_mod__decode_kernel(
    A_x, A_c_kv, A_w_q, A_w_uk, A_w_uv, A_w_o, B_x, B_w_r, B_w_gate, B_w_up, B_w_down,
):
    return _make()(A_x, A_c_kv, A_w_q, A_w_uk, A_w_uv, A_w_o, B_x, B_w_r, B_w_gate, B_w_up, B_w_down)
```

```python
import jax
import jax.numpy as jnp
from jax import lax
import jax.experimental.pallas as pl
import jax.experimental.pallas.tpu as pltpu

bf16, f32, i32 = jnp.bfloat16, jnp.float32, jnp.int32

LANES = 128
ROWS = 8
G = 16
LOG_G = 4
Q_CHUNK = 64
BULK_HEADS = 2
TAIL_HEADS = 8


def _dot(a, b):
    return jnp.dot(a, b, preferred_element_type=f32)


def _dot_nt(a, b):
    return lax.dot_general(a, b, (((1,), (1,)), ((), ())), preferred_element_type=f32)


def _sigmoid(v):
    return 1.0 / (1.0 + jnp.exp(-v))


def _iotas(shape):
    return lax.broadcasted_iota(i32, shape, 0), lax.broadcasted_iota(i32, shape, 1)


def _same_head(shape):
    r, c = _iotas(shape)
    return (r & (G - 1)) == (c & (G - 1))


def _one_hot(cond):
    return jnp.where(cond, 1.0, 0.0).astype(bf16)


def _kernel(x_h, ckv_h, wq_h, wuk_h, wuv_h, wo_h, wr_h, wg_h, wu_h, wd_h, o_ref,
            x_v, wr_v, ckv_v, wq_v, wuk_v, wuv_v, wg_v, wu_v, wd_v,
            wo_bulk_v, wo_edge_v, wo_tail_v,
            spread_v, gather_v, xq_v, qa_v, lat_v, ctx_v):
    B, M = x_v.shape
    _, H, D = wq_v.shape
    DC = ckv_v.shape[2]
    groups = range(H // G)
    n_bulk = wo_bulk_v.shape[0]
    h_tail = H - TAIL_HEADS
    m_full = wo_tail_v.shape[1]
    m_down = m_full - LANES

    def body(sems):
        copy = pltpu.make_async_copy
        cp_x = copy(x_h, x_v, sems.at[0])
        cp_wr = copy(wr_h, wr_v, sems.at[1])
        cp_wq = copy(wq_h, wq_v, sems.at[2])
        cp_wuk = copy(wuk_h, wuk_v, sems.at[3])
        cp_ckv = copy(ckv_h, ckv_v, sems.at[4])
        cp_wuv = copy(wuv_h, wuv_v, sems.at[5])
        cp_wg = copy(wg_h, wg_v, sems.at[6])
        cp_wu = copy(wu_h, wu_v, sems.at[7])
        lo, hi = pl.ds(0, m_down), pl.ds(m_down, M - m_down)
        cp_wd_lo = copy(wd_h.at[lo], wd_v.at[lo], sems.at[8])
        cp_wd_hi = copy(wd_h.at[hi], wd_v.at[hi], sems.at[9])
        cp_edge = copy(wo_h.at[pl.ds(h_tail, TAIL_HEADS), pl.ds(m_full, M - m_full)],
                       wo_edge_v, sems.at[10])

        def cp_bulk(i):
            return copy(wo_h.at[pl.ds(i * BULK_HEADS, BULK_HEADS)], wo_bulk_v.at[i],
                        sems.at[11 + i])

        def cp_tail(i):
            return copy(wo_h.at[h_tail + i, pl.ds(0, m_full)], wo_tail_v.at[i],
                        sems.at[11 + n_bulk + i])

        for cp in ([cp_x, cp_wr, cp_wq, cp_wuk, cp_ckv, cp_wuv, cp_wg, cp_wu,
                    cp_wd_lo, cp_wd_hi, cp_edge]
                   + [cp_bulk(i) for i in range(n_bulk)]
                   + [cp_tail(i) for i in range(TAIL_HEADS)]):
            cp.start()

        r, c = _iotas(spread_v.shape)
        spread_v[...] = _one_hot(r == (c >> LOG_G))
        r, c = _iotas(gather_v.shape)
        gather_v[...] = _one_hot(c == (r >> LOG_G))

        cp_x.wait()
        cp_wr.wait()
        x = jnp.concatenate([x_v[...].astype(f32), jnp.zeros((ROWS - B, M), f32)], axis=0)
        xc = x - jnp.mean(x, axis=-1, keepdims=True)
        var = jnp.mean(xc * xc, axis=-1, keepdims=True)
        xn_lo = (xc / jnp.sqrt(var + 1e-5)).astype(bf16)
        xn = xn_lo.astype(f32)
        wr = wr_v[...].astype(f32).reshape(1, M)
        route = _sigmoid(jnp.sum(xn * wr, axis=-1, keepdims=True))

        for m0 in range(0, M, LANES):
            n = min(LANES, M - m0)
            xe = _dot(xn_lo[:, m0:m0 + n], spread_v[0:n, 0:n * G])
            keep = _same_head((G, n * G))
            for b in range(B):
                v = jnp.where(keep, jnp.broadcast_to(xe[b:b + 1], (G, n * G)), 0.0)
                xq_v[b * G:(b + 1) * G, m0 * G:(m0 + n) * G] = v.astype(bf16)

        cp_wq.wait()

        def q_step(i, acc):
            rows = pl.ds(pl.multiple_of(i * Q_CHUNK, Q_CHUNK), Q_CHUNK)
            lhs = xq_v[:, pl.ds(pl.multiple_of(i * Q_CHUNK * G, Q_CHUNK * G), Q_CHUNK * G)]
            return tuple(
                acc[g] + _dot(lhs, wq_v[rows, g * G:(g + 1) * G, :].reshape(Q_CHUNK * G, D))
                for g in groups)

        zeros = tuple(jnp.zeros((B * G, D), f32) for _ in groups)
        q = [t.astype(bf16) for t in lax.fori_loop(0, M // Q_CHUNK, q_step, zeros)]

        cp_wuk.wait()

        def qa_step(i, carry):
            cols = pl.ds(pl.multiple_of(i * LANES, LANES), LANES)
            t = jnp.concatenate(
                [_dot_nt(q[g], wuk_v[cols, g * G:(g + 1) * G, :].reshape(LANES * G, D))
                 for g in groups], axis=0)
            t = jnp.where(_same_head(t.shape), t, 0.0).astype(bf16)
            qa_v[:, cols] = _dot(t, gather_v[...]).astype(bf16)
            return carry

        lax.fori_loop(0, DC // LANES, qa_step, 0)

        cp_ckv.wait()

        def attn_step(b, carry):
            rows = [pl.ds(pl.multiple_of((g * B + b) * G, G), G) for g in groups]
            qa = jnp.concatenate([qa_v[rs, :] for rs in rows], axis=0)
            s = _dot_nt(qa, ckv_v[b]) * (D ** -0.5)
            p = jnp.exp(s - jnp.max(s, axis=-1, keepdims=True))
            lat = _dot(p.astype(bf16), ckv_v[b]) / jnp.sum(p, axis=-1, keepdims=True)
            lat = lat.astype(bf16)
            for g in groups:
                lat_v[rows[g], :] = lat[g * G:(g + 1) * G]
            return carry

        lax.fori_loop(0, B, attn_step, 0)

        cp_wuv.wait()

        def ctx_step(i, acc):
            cols = pl.ds(pl.multiple_of(i * LANES, LANES), LANES)
            t = _dot(lat_v[:, cols], spread_v[...])
            t = jnp.where(_same_head(t.shape), t, 0.0).astype(bf16)
            return tuple(
                acc[g] + _dot(t[g * B * G:(g + 1) * B * G],
                              wuv_v[cols, g * G:(g + 1) * G, :].reshape(LANES * G, D))
                for g in groups)

        ctx = jnp.concatenate(lax.fori_loop(0, DC // LANES, ctx_step, zeros), axis=0)
        r, c = _iotas((H * ROWS, B * H))
        h, b = r >> 3, r & (ROWS - 1)
        src = jnp.where(b < B, ((h >> LOG_G) * B + b) * G + (h & (G - 1)), -1)
        ctx_v[...] = _dot(_one_hot(c == src), ctx.astype(bf16)).reshape(H, ROWS, D).astype(bf16)

        cp_wg.wait()
        gate = _dot(xn_lo, wg_v[...])
        cp_wu.wait()
        hid = (gate * _sigmoid(gate) * _dot(xn_lo, wu_v[...])).astype(bf16)
        cp_wd_lo.wait()
        y_lo = _dot_nt(hid, wd_v[lo, :])
        cp_wd_hi.wait()
        y = jnp.concatenate([y_lo, _dot_nt(hid, wd_v[hi, :])], axis=1)
        z = xn + (xn * 0.0 + y * route)
        gain = z * _sigmoid(z)

        cp_edge.wait()
        s_edge = _dot_nt(
            jnp.concatenate([ctx_v[h_tail + i] for i in range(TAIL_HEADS)], axis=1),
            jnp.concatenate([wo_edge_v[i] for i in range(TAIL_HEADS)], axis=1))

        def bulk_step(i, acc):
            cp_bulk(i).wait()
            return acc + _dot_nt(
                jnp.concatenate([ctx_v[i * BULK_HEADS + j] for j in range(BULK_HEADS)], axis=1),
                jnp.concatenate([wo_bulk_v[i, j] for j in range(BULK_HEADS)], axis=1))

        s_bulk = lax.fori_loop(0, n_bulk, bulk_step, jnp.zeros((ROWS, M), f32))
        edge = x[:, m_full:] + (s_bulk[:, m_full:] + s_edge) * gain[:, m_full:]
        o_ref[:, m_full:] = edge[:B].astype(o_ref.dtype)

        def tail_step(i, acc):
            cp_tail(i).wait()
            acc = acc + _dot_nt(ctx_v[h_tail + i], wo_tail_v[i]) * gain[:, :m_full]
            for m0 in range(0, m_full, LANES):
                o_ref[:, m0:m0 + LANES] = acc[:B, m0:m0 + LANES].astype(o_ref.dtype)
            return acc

        lax.fori_loop(0, TAIL_HEADS, tail_step,
                      x[:, :m_full] + s_bulk[:, :m_full] * gain[:, :m_full])

    pl.run_scoped(body, pltpu.SemaphoreType.DMA((11 + n_bulk + TAIL_HEADS,)))


@jax.jit
def pallas_recurrent_scan__compressed_kv_cla__moe_arch_mod__decode_kernel(
    A_x: jax.Array,
    A_c_kv: jax.Array,
    A_w_q: jax.Array,
    A_w_uk: jax.Array,
    A_w_uv: jax.Array,
    A_w_o: jax.Array,
    B_x: jax.Array,
    B_w_r: jax.Array,
    B_w_gate: jax.Array,
    B_w_up: jax.Array,
    B_w_down: jax.Array,
):
    del B_x
    B, Sq, M = A_x.shape
    _, H, D = A_w_q.shape
    DC = A_c_kv.shape[2]
    assert Sq == 1 and B <= ROWS and H % G == 0 and D == LANES and DC % LANES == 0
    assert M % Q_CHUNK == 0 and M % LANES != 0 and (H - TAIL_HEADS) % BULK_HEADS == 0
    m_full = M // LANES * LANES

    w_o_t = jnp.transpose(A_w_o, (0, 2, 1))
    w_down_t = B_w_down.T
    out = pl.pallas_call(
        _kernel,
        in_specs=[pl.BlockSpec(memory_space=pltpu.HBM)] * 10,
        out_shape=jax.ShapeDtypeStruct((B, M), A_x.dtype),
        scratch_shapes=[
            pltpu.VMEM((B, M), A_x.dtype),
            pltpu.VMEM(B_w_r.shape, B_w_r.dtype),
            pltpu.VMEM(A_c_kv.shape, A_c_kv.dtype),
            pltpu.VMEM(A_w_q.shape, A_w_q.dtype),
            pltpu.VMEM(A_w_uk.shape, A_w_uk.dtype),
            pltpu.VMEM(A_w_uv.shape, A_w_uv.dtype),
            pltpu.VMEM(B_w_gate.shape, B_w_gate.dtype),
            pltpu.VMEM(B_w_up.shape, B_w_up.dtype),
            pltpu.VMEM(w_down_t.shape, w_down_t.dtype),
            pltpu.VMEM(((H - TAIL_HEADS) // BULK_HEADS, BULK_HEADS, M, D), w_o_t.dtype),
            pltpu.VMEM((TAIL_HEADS, M - m_full, D), w_o_t.dtype),
            pltpu.VMEM((TAIL_HEADS, m_full, D), w_o_t.dtype),
            pltpu.VMEM((LANES, LANES * G), bf16),
            pltpu.VMEM((LANES * G, LANES), bf16),
            pltpu.VMEM((B * G, M * G), bf16),
            pltpu.VMEM((B * H, DC), bf16),
            pltpu.VMEM((B * H, DC), bf16),
            pltpu.VMEM((H, ROWS, D), bf16),
        ],
        compiler_params=pltpu.CompilerParams(vmem_limit_bytes=100 * 1024 * 1024),
    )(A_x.reshape(B, M), A_c_kv, A_w_q, A_w_uk, A_w_uv, w_o_t,
      B_w_r, B_w_gate, B_w_up, w_down_t)
    return out.reshape(B, Sq, M)
```
